```python
import os as _os
_os.environ.setdefault("JAX_PLATFORMS", "cpu")
import jax
import jax.numpy as jnp

def _softmax(x, axis=-1):
    return jax.nn.softmax(x, axis=axis)
def _gelu(x):
    return jax.nn.gelu(x, approximate=True)
def _silu(x):
    return jax.nn.silu(x)
def _sigmoid(x):
    return jax.nn.sigmoid(x)
def _layernorm(x, axis=-1, eps=1e-5):
    m = jnp.mean(x, axis=axis, keepdims=True)
    v = jnp.var(x, axis=axis, keepdims=True)
    return (x - m) / jnp.sqrt(v + eps)
def _scatter_add(tgt, idx, src, axis=0):
    return tgt.at[idx].add(src)
def _segment_sum(src, seg, n):
    return jax.ops.segment_sum(src, seg, n)
class _Rng:
    def __init__(self, key):
        self._k = key
    def _next(self):
        self._k, sub = jax.random.split(self._k)
        return sub
    def normal(self, shape):
        return jax.random.normal(self._next(), shape, dtype=jnp.bfloat16)
    def randint(self, lo, hi, shape):
        return jax.random.randint(self._next(), shape, lo, hi, dtype=jnp.int32)
    def uniform(self, shape, lo=0.0, hi=1.0):
        return jax.random.uniform(self._next(), shape, jnp.bfloat16, lo, hi)
    def permutation(self, n):
        return jax.random.permutation(self._next(), n)


kernel_name = 'concat_heads__ssm_conv_h3__sliding_block__prompt'

def setup_inputs():
    _rng = _Rng(jax.random.key(int.from_bytes(__import__("os").urandom(4), "little")))
    _w = (lambda a: (lambda t: t.astype(jnp.bfloat16) if jnp.issubdtype(t.dtype, jnp.floating) else t)(jnp.asarray(a)))
    def _A_setup():
        B, S, D = 1, 2048, 512
        ks = 4
        return {
            "q": _w((lambda *s: _rng.normal(s) * 0.05)(B, S, D)),
            "k": _w((lambda *s: _rng.normal(s) * 0.2)(B, S, D)),
            "v": _w((lambda *s: _rng.normal(s) * 0.2)(B, S, D)),
            "shift_k": _w((lambda *s: _rng.normal(s) * 0.2)(D, ks) * 0.5),
            "ssm_k": _w((lambda *s: _rng.normal(s) * 0.2)(D, S) * (1.0 / S ** 0.5)),
            "ssm_D": _w((lambda *s: _rng.normal(s) * 0.2)(D)),
        }
    _A_in = _A_setup()

    def _B_setup():
        B, S, D = 1, 2048, 512
        return {
            "x": _w((lambda *s: _rng.normal(s) * 0.2)(B, S, D)),
            "wqkv": _w((lambda *s: _rng.normal(s) * 0.2)(D, 3 * D)),
            "wo": _w((lambda *s: _rng.normal(s) * 0.05)(D, D)),
        }
    _B_in = _B_setup()

    return {
        "A_q": _A_in["q"],
        "A_k": _A_in["k"],
        "A_v": _A_in["v"],
        "A_shift_k": _A_in["shift_k"],
        "A_ssm_k": _A_in["ssm_k"],
        "A_ssm_D": _A_in["ssm_D"],
        "B_x": _B_in["x"],
        "B_wqkv": _B_in["wqkv"],
        "B_wo": _B_in["wo"],
    }

def reference(A_q, A_k, A_v, A_shift_k, A_ssm_k, A_ssm_D, B_x, B_wqkv, B_wo):
    def _A_ref(q, k, v, shift_k, ssm_k, ssm_D):
        B, S, D = q.shape
        ks = shift_k.shape[-1]
        k_pad = jnp.pad(k, ((0, 0), (ks - 1, 0), (0, 0)))
        k_shift = jnp.zeros_like(k)
        for t in range(ks):
            k_shift = k_shift + k_pad[:, t:t + S, :] * shift_k[:, ks - 1 - t][None, None, :]
        kv = k_shift * v
        L = 2 * S
        kv_pad = jnp.pad(kv, ((0, 0), (0, S), (0, 0)))
        kf_pad = jnp.pad(ssm_k, ((0, 0), (0, S)))
        kv_f = (lambda x, axes=(-2,-1): jnp.fft.rfft2(x.astype(jnp.float32), axes=axes))(kv_pad[:, None, :, :], axes=(1, 2))
        kf_f = (lambda x, axes=(-2,-1): jnp.fft.rfft2(x.astype(jnp.float32), axes=axes))(kf_pad[:, None, :], axes=(1, 2))
        kf_f = (lambda x, *d: x.transpose(*d))(kf_f, 1, 2, 0)
        y_f = kv_f * kf_f[None, :, :, :]
        y = (lambda x, s, axes=(-2,-1): jnp.fft.irfft2(x, s=s, axes=axes).astype(jnp.bfloat16))(y_f, (1, L), axes=(1, 2))[:, 0, :S, :]
        y = y + kv * ssm_D[None, None, :]
        return q * y

    def _B_ref(x, wqkv, wo):
        B, S, D = x.shape
        H = 32; Dh = D // H; W = 256
        qkv = (lambda x, *d: x.transpose(*d))((x @ wqkv).reshape(B, S, 3, H, Dh), 2, 0, 3, 1, 4)
        q, k, v = qkv[0], qkv[1], qkv[2]
        scores = jnp.einsum("bhqd,bhkd->bhqk", q, k) * (Dh ** -0.5)
        idx = jnp.arange(S)
        mask = (idx[:, None] - idx[None, :] >= 0) & (idx[:, None] - idx[None, :] < W)
        scores = jnp.where(mask[None, None], scores, -1e9)
        p = _softmax(scores, axis=-1)
        o = jnp.einsum("bhqk,bhkd->bhqd", p, v)
        return (lambda x, *d: x.transpose(*d))(o, 0, 2, 1, 3).reshape(B, S, D) @ wo

    a = _A_ref(A_q, A_k, A_v, A_shift_k, A_ssm_k, A_ssm_D)
    b = _B_ref(B_x, B_wqkv, B_wo)
    return jnp.concatenate([a, b], axis=-1)
```

```python
import jax
import jax.numpy as jnp
import numpy as np
import jax.experimental.pallas as pl
import jax.experimental.pallas.tpu as pltpu

_C = 128
_NT = (((1,), (1,)), ((), ()))
_TN = (((0,), (0,)), ((), ()))
_F32 = jnp.float32
_BF16 = jnp.bfloat16


def _dft_mats():
    c = _C
    w = np.pi * (2 * np.arange(c) + 1) / (2 * c)
    ang = w[:, None] * np.arange(c)[None, :]
    fwd = np.concatenate([np.cos(ang), -np.sin(ang)], 0)
    inv = np.concatenate([np.cos(ang).T, -np.sin(ang).T], 1) / c
    return fwd.astype(np.float32), inv.astype(np.float32)


def _kernel(q_ref, k_ref, v_ref, sh_ref, h_ref, d_ref, x_ref, wqkv_ref, wo_ref,
            fwd_ref, inv_ref, o_ref,
            kbuf, xs, hs, gprev, kscr, vt, ot, yh, qsc):
    i = pl.program_id(0)
    c = _C

    @pl.when(i == 0)
    def _():
        kbuf[0:8, :] = jnp.zeros((8, 512), _F32)
        xs[16] = jnp.zeros(gprev.shape, _F32)
        hs[16] = jnp.zeros(gprev.shape, _F32)
        gprev[...] = jnp.zeros(gprev.shape, _F32)
        kscr[0:256, :] = jnp.zeros((256, 512), _BF16)
        vt[0:2] = jnp.zeros((2, 512, 128), _BF16)

    kbuf[8:136, :] = k_ref[...].astype(_F32)
    sh = sh_ref[...].astype(_F32)
    ks = kbuf[8:136, :] * sh[0:1, :]
    for j in range(1, 4):
        ks = ks + kbuf[8 - j:136 - j, :] * sh[j:j + 1, :]
    kbuf[0:8, :] = kbuf[128:136, :]
    kv = ks * v_ref[...].astype(_F32)
    fwd = fwd_ref[...]
    xs[i] = jnp.dot(fwd, kv.astype(_BF16), preferred_element_type=_F32)
    g = jax.lax.dot_general(fwd, h_ref[...], _NT, preferred_element_type=_F32)
    sgn = (1 - 2 * (jax.lax.broadcasted_iota(jnp.int32, (c, 512), 0) & 1)).astype(_F32)
    gp = gprev[...]
    hs[i, 0:c, :] = g[0:c] - sgn * gp[c:]
    hs[i, c:, :] = g[c:] + sgn * gp[0:c]
    gprev[...] = g

    NS = 8
    hidx = [jnp.where(m <= i, m, 16) for m in range(NS)]
    xidx = [jnp.where(m <= i, i - m, 16) for m in range(NS)]

    def mac(t):
        r = (t // 2) * 8
        ln = slice((t % 2) * 256, (t % 2) * 256 + 256)
        ar = ai = None
        for m in range(NS):
            hr = hs[hidx[m], r:r + 8, ln]
            hi = hs[hidx[m], c + r:c + r + 8, ln]
            xr = xs[xidx[m], r:r + 8, ln]
            xi = xs[xidx[m], c + r:c + r + 8, ln]
            tr = hr * xr - hi * xi
            ti = hr * xi + hi * xr
            ar, ai = (tr, ti) if m == 0 else (ar + tr, ai + ti)
        yh[r:r + 8, ln] = ar
        yh[c + r:c + r + 8, ln] = ai

    base = pl.multiple_of(i * c, c)
    xb = x_ref[...]
    nm = 0
    for j in range(12):
        cs = slice(j * 128, j * 128 + 128)
        pj = jnp.dot(xb, wqkv_ref[:, cs], preferred_element_type=_F32)
        l0 = (j % 4) * 128
        if j < 4:
            qsc[:, l0:l0 + 128] = (pj * (0.25 * 1.4426950408889634)).astype(_BF16)
        elif j < 8:
            kscr[pl.ds(base + 256, c), l0:l0 + 128] = pj.astype(_BF16)
        else:
            vt[i + 2, l0:l0 + 128, :] = pj.T.astype(_BF16)
        while nm < (j + 1) * 32 // 12:
            mac(nm)
            nm += 1

    @pl.when(i >= NS)
    def _():
        R = 16
        for r in range(0, c, R):
            def body(m, acc):
                ar, ai = acc
                hr = hs[m, r:r + R, :]
                hi = hs[m, c + r:c + r + R, :]
                xr = xs[i - m, r:r + R, :]
                xi = xs[i - m, c + r:c + r + R, :]
                return ar + (hr * xr - hi * xi), ai + (hr * xi + hi * xr)
            ar, ai = jax.lax.fori_loop(
                NS, i + 1, body, (yh[r:r + R, :], yh[c + r:c + r + R, :]))
            yh[r:r + R, :] = ar
            yh[c + r:c + r + R, :] = ai

    kidx = jax.lax.broadcasted_iota(jnp.int32, (c, c), 0)
    qidx = jax.lax.broadcasted_iota(jnp.int32, (c, c), 1)
    m1 = kidx > qidx
    bias02 = jnp.where(m1 & (i < 2), -1e30, 0.0).astype(_F32)
    bias1 = jnp.where(i < 1, -1e30, 0.0).astype(_F32)
    i32 = jnp.int32
    mhi = pltpu.bitcast(jnp.where(m1, -1, 0).astype(jnp.int16), i32)
    mlo = ~mhi
    lane_h = jax.lax.broadcasted_iota(i32, (c // 2, c), 1) >> 4
    qsi = pltpu.bitcast(qsc[...], i32)

    def qk(h):
        g0 = (h // 8) * 128
        kw = kscr[pl.ds(base, 384), g0:g0 + 128]
        qm = pltpu.bitcast(jnp.where(lane_h == h % 8, qsi[:, g0:g0 + 128], 0), _BF16)
        s = jax.lax.dot_general(kw, qm, _NT, preferred_element_type=_F32)
        return jnp.where(m1, s[0:128] + bias02, s[256:384]), s[128:256] + bias1

    def sm(ss):
        s02, s1 = ss
        m = jnp.max(jnp.maximum(s02, s1), axis=0, keepdims=True)
        p02 = jnp.exp2(s02 - m)
        p1 = jnp.exp2(s1 - m)
        l = jnp.sum(p02 + p1, axis=0, keepdims=True)
        pi = pltpu.bitcast(p02.astype(_BF16), i32)
        return (pltpu.bitcast(pi & mhi, _BF16), p1.astype(_BF16),
                pltpu.bitcast(pi & mlo, _BF16), 1.0 / l)

    def pv(h, pp):
        rows = slice(h * 16, h * 16 + 16)
        o = (jnp.dot(vt[i, rows, :], pp[0], preferred_element_type=_F32)
             + jnp.dot(vt[i + 1, rows, :], pp[1], preferred_element_type=_F32)
             + jnp.dot(vt[i + 2, rows, :], pp[2], preferred_element_type=_F32))
        ot[rows, :] = o * pp[3]

    LA, LB = 6, 4
    S_, P_ = {}, {}
    for t in range(32 + LA + LB):
        if t < 32:
            S_[t] = qk(t)
        if 0 <= t - LA < 32:
            P_[t - LA] = sm(S_.pop(t - LA))
        if 0 <= t - LA - LB < 32:
            pv(t - LA - LB, P_.pop(t - LA - LB))
    y = jnp.dot(inv_ref[...], yh[...].astype(_BF16), preferred_element_type=_F32)
    y = y + kv * d_ref[...].astype(_F32)
    o_ref[:, 0:512] = (q_ref[...].astype(_F32) * y).astype(_BF16)
    o_ref[:, 512:1024] = jnp.dot(ot[...].T.astype(_BF16), wo_ref[...],
                                 preferred_element_type=_F32).astype(_BF16)


@jax.jit
def pallas_concat_heads__ssm_conv_h3__sliding_block__prompt_kernel(
    A_q, A_k, A_v, A_shift_k, A_ssm_k, A_ssm_D, B_x, B_wqkv, B_wo,
):
    B, S, D = A_q.shape
    c = _C
    n = S // c
    fwd, inv = _dft_mats()
    fwd = jnp.asarray(fwd, _BF16)
    inv = jnp.asarray(inv, _BF16)
    row = pl.BlockSpec((c, D), lambda i: (i, 0))
    full = lambda shp: pl.BlockSpec(shp, lambda i: (0,) * len(shp))
    out = pl.pallas_call(
        _kernel,
        grid=(n,),
        in_specs=[row, row, row, full((4, D)), pl.BlockSpec((D, c), lambda i: (0, i)),
                  full((1, D)), row, full((D, 3 * D)), full((D, D)),
                  full((2 * c, c)), full((c, 2 * c))],
        out_specs=pl.BlockSpec((c, 2 * D), lambda i: (i, 0)),
        out_shape=jax.ShapeDtypeStruct((S, 2 * D), _BF16),
        scratch_shapes=[
            pltpu.VMEM((136, D), _F32),
            pltpu.VMEM((n + 1, 2 * c, D), _F32),
            pltpu.VMEM((n + 1, 2 * c, D), _F32),
            pltpu.VMEM((2 * c, D), _F32),
            pltpu.VMEM((S + 256, D), _BF16),
            pltpu.VMEM((n + 2, D, c), _BF16),
            pltpu.VMEM((D, c), _F32),
            pltpu.VMEM((2 * c, D), _F32),
            pltpu.VMEM((c, D), _BF16),
        ],
        compiler_params=pltpu.CompilerParams(
            dimension_semantics=("arbitrary",), vmem_limit_bytes=64 * 1024 * 1024),
    )(A_q[0], A_k[0], A_v[0], A_shift_k.T, A_ssm_k, A_ssm_D.reshape(1, D),
      B_x[0], B_wqkv, B_wo, fwd, inv)
    return out.reshape(B, S, 2 * D)
```
